```python
import os as _os
_os.environ.setdefault("JAX_PLATFORMS", "cpu")
import jax
import jax.numpy as jnp

def _softmax(x, axis=-1):
    return jax.nn.softmax(x, axis=axis)
def _gelu(x):
    return jax.nn.gelu(x, approximate=True)
def _silu(x):
    return jax.nn.silu(x)
def _sigmoid(x):
    return jax.nn.sigmoid(x)
def _layernorm(x, axis=-1, eps=1e-5):
    m = jnp.mean(x, axis=axis, keepdims=True)
    v = jnp.var(x, axis=axis, keepdims=True)
    return (x - m) / jnp.sqrt(v + eps)
def _scatter_add(tgt, idx, src, axis=0):
    return tgt.at[idx].add(src)
def _segment_sum(src, seg, n):
    return jax.ops.segment_sum(src, seg, n)
class _Rng:
    def __init__(self, key):
        self._k = key
    def _next(self):
        self._k, sub = jax.random.split(self._k)
        return sub
    def normal(self, shape):
        return jax.random.normal(self._next(), shape, dtype=jnp.bfloat16)
    def randint(self, lo, hi, shape):
        return jax.random.randint(self._next(), shape, lo, hi, dtype=jnp.int32)
    def uniform(self, shape, lo=0.0, hi=1.0):
        return jax.random.uniform(self._next(), shape, jnp.bfloat16, lo, hi)
    def permutation(self, n):
        return jax.random.permutation(self._next(), n)


kernel_name = 'sequential_preLN__mha_block__swiglu_ffn__prompt'

def setup_inputs():
    _rng = _Rng(jax.random.key(int.from_bytes(__import__("os").urandom(4), "little")))
    _w = (lambda a: (lambda t: t.astype(jnp.bfloat16) if jnp.issubdtype(t.dtype, jnp.floating) else t)(jnp.asarray(a)))
    def _A_setup():
        B, S, D, H = 1, 2048, 640, 32
        return {
            "x": _w((lambda *s: _rng.normal(s) * 0.05)(B, S, D)),
            "wqkv": _w((lambda *s: _rng.normal(s) * 0.05)(D, 3 * D)),
            "wo": _w((lambda *s: _rng.normal(s) * 0.05)(D, D)),
        }
    _A_in = _A_setup()

    def _B_setup():
        B, S, D, F = 1, 2048, 640, 1728
        return {
            "x": _w((lambda *s: _rng.normal(s) * 0.05)(B, S, D)),
            "w_gate": _w((lambda *s: _rng.normal(s) * 0.05)(D, F)),
            "w_up": _w((lambda *s: _rng.normal(s) * 0.05)(D, F)),
            "w_down": _w((lambda *s: _rng.normal(s) * 0.05)(F, D)),
        }
    _B_in = _B_setup()

    return {
        "A_x": _A_in["x"],
        "A_wqkv": _A_in["wqkv"],
        "A_wo": _A_in["wo"],
        "B_x": _B_in["x"],
        "B_w_gate": _B_in["w_gate"],
        "B_w_up": _B_in["w_up"],
        "B_w_down": _B_in["w_down"],
    }

def reference(A_x, A_wqkv, A_wo, B_x, B_w_gate, B_w_up, B_w_down):
    def _A_ref(x, wqkv, wo):
        B, S, D = x.shape
        H = 32
        Dh = D // H
        qkv = (lambda x, *d: x.transpose(*d))((x @ wqkv).reshape(B, S, 3, H, Dh), 2, 0, 3, 1, 4)
        q, k, v = qkv[0], qkv[1], qkv[2]
        scores = jnp.einsum("bhqd,bhkd->bhqk", q, k) * (Dh ** -0.5)
        p = _softmax(scores, axis=-1)
        o = jnp.einsum("bhqk,bhkd->bhqd", p, v)
        return (lambda x, *d: x.transpose(*d))(o, 0, 2, 1, 3).reshape(B, S, D) @ wo

    def _B_ref(x, w_gate, w_up, w_down):
        g = _silu(x @ w_gate)
        u = x @ w_up
        return (g * u) @ w_down

    x = A_x
    h = x + _A_ref(_layernorm(x, axis=-1), A_wqkv, A_wo)
    h2 = h + _B_ref(_layernorm(h, axis=-1), B_w_gate, B_w_up, B_w_down)
    return h2
```

```python
import functools

import jax
import jax.numpy as jnp
import numpy as np
from jax import lax
import jax.experimental.pallas as pl
import jax.experimental.pallas.tpu as pltpu

H = 32
DH = 20
EPS = 1e-5
LOG2E = 1.4426950408889634
L_LO = 2.0 ** -60
L_HI = 2.0 ** 60

RB1 = 512
RB3 = 512
BQ = 1024
KC = 256
BQS = 256

f32 = jnp.float32
bf16 = jnp.bfloat16


def _mm(a, b):
    return lax.dot_general(a, b, (((1,), (0,)), ((), ())), preferred_element_type=f32)


def _mm_nt(a, b):
    return lax.dot_general(a, b, (((1,), (1,)), ((), ())), preferred_element_type=f32)


def _layernorm(x):
    m = jnp.mean(x, axis=-1, keepdims=True)
    d = x - m
    v = jnp.mean(d * d, axis=-1, keepdims=True)
    return d * lax.rsqrt(v + EPS)


def _kernel(x_hbm, wqkv_hbm, wo_hbm, wg_hbm, wu_hbm, wd_hbm, out_hbm,
            x_v, wqkv_v, wo_v, wg_v, wu_v, wd_v,
            wqvt_v, k_v, qt_v, vt_v, kr_v, ot_v, out_v,
            in_sems, out_sems):
    S, D = x_v.shape

    cp_x = pltpu.make_async_copy(x_hbm, x_v, in_sems.at[0])
    cp_wqkv = pltpu.make_async_copy(wqkv_hbm, wqkv_v, in_sems.at[1])
    cp_rest = [
        pltpu.make_async_copy(wo_hbm, wo_v, in_sems.at[2]),
        pltpu.make_async_copy(wg_hbm, wg_v, in_sems.at[3]),
        pltpu.make_async_copy(wu_hbm, wu_v, in_sems.at[4]),
        pltpu.make_async_copy(wd_hbm, wd_v, in_sems.at[5]),
    ]
    cp_wqkv.start()
    cp_x.start()
    cp_wqkv.wait()
    for c in cp_rest:
        c.start()

    wqvt_v[0:D, :] = wqkv_v[:, 0:D].astype(f32).T.astype(bf16)
    wqvt_v[D:2 * D, :] = wqkv_v[:, 2 * D:3 * D].astype(f32).T.astype(bf16)
    cp_x.wait()

    qscale = (DH ** -0.5) * LOG2E
    row8 = lax.broadcasted_iota(jnp.int32, (8, RB1), 0)

    def p1(i, carry):
        r0 = pl.multiple_of(i * RB1, RB1)
        xn = _layernorm(x_v[pl.ds(r0, RB1), :].astype(f32)).astype(bf16)
        k = _mm(xn, wqkv_v[:, D:2 * D]).astype(bf16)
        for t in range(D // 128):
            k_v[t, pl.ds(r0, RB1), :] = k[:, t * 128:(t + 1) * 128]
        qvt = _mm_nt(wqvt_v[...], xn)
        qt = qvt[0:D] * qscale
        vt = qvt[D:2 * D]
        zeros8 = jnp.zeros((8, RB1), f32)
        for p in range(H // 2):
            a = 2 * DH * p
            q_mid = qt[a + 16:a + 24]
            q_even = jnp.concatenate(
                [qt[a:a + 16], jnp.where(row8 < 4, q_mid, 0.0), zeros8], axis=0)
            q_odd = jnp.concatenate(
                [jnp.where(row8 >= 4, q_mid, 0.0), qt[a + 24:a + 40], zeros8], axis=0)
            qt_v[2 * p, :, pl.ds(r0, RB1)] = q_even.astype(bf16)
            qt_v[2 * p + 1, :, pl.ds(r0, RB1)] = q_odd.astype(bf16)
            v_mid = vt[a + 16:a + 24]
            vt_v[2 * p, :, pl.ds(r0, RB1)] = jnp.concatenate(
                [vt[a:a + 16], jnp.where(row8 < 4, v_mid, 1.0)], axis=0)
            vt_v[2 * p + 1, :, pl.ds(r0, RB1)] = jnp.concatenate(
                [jnp.where(row8 >= 4, v_mid, 1.0), vt[a + 24:a + 40]], axis=0)
        return carry

    lax.fori_loop(0, S // RB1, p1, 0)

    lane = lax.broadcasted_iota(jnp.int32, (S // 2, 128), 1)

    def roll_keys(p, odd):
        a = 2 * DH * p + (16 if odd else 0)
        t = a // 128
        off = a % 128
        t2 = jnp.minimum(t + 1, D // 128 - 1)
        k0 = pltpu.bitcast(k_v[t], jnp.uint32)
        k1 = pltpu.bitcast(k_v[t2], jnp.uint32)
        kw = jnp.where(lane >= off, k0, k1)
        kw = pltpu.roll(kw, (128 - off) % 128, 1)
        kr_v[int(odd)] = pltpu.bitcast(kw, bf16)

    def merge(o_e, o_o):
        l_e = o_e[20:21]
        l_o = o_o[0:1]
        n_e = o_e * (1.0 / l_e)
        n_o = o_o * (1.0 / l_o)
        r8 = lax.broadcasted_iota(jnp.int32, (8, o_e.shape[1]), 0)
        mid = jnp.where(r8 < 4, n_e[16:24], n_o[0:8])
        o = jnp.concatenate([n_e[0:16], mid, n_o[8:24]], axis=0)
        return o, l_e, l_o

    def fast(p, bad):
        roll_keys(p, False)
        roll_keys(p, True)
        r0 = pl.multiple_of(p * (2 * DH), 8)
        nk = S // KC
        items = [(qb, e, j) for qb in range(S // BQ) for e in range(2) for j in range(nk)]

        def scores(it):
            qb, e, j = it
            return _mm(kr_v[e, j * KC:(j + 1) * KC, 0:32],
                       qt_v[2 * p + e, :, qb * BQ:(qb + 1) * BQ])

        s = scores(items[0])
        accs = {}
        for n, (qb, e, j) in enumerate(items):
            s_next = scores(items[n + 1]) if n + 1 < len(items) else None
            pt = jnp.exp2(s).astype(bf16)
            o = _mm(vt_v[2 * p + e, :, j * KC:(j + 1) * KC], pt)
            accs[e] = o if j == 0 else accs[e] + o
            s = s_next
            if e == 1 and j == nk - 1:
                oo, l_e, l_o = merge(accs[0], accs[1])
                ot_v[pl.ds(r0, 2 * DH), qb * BQ:(qb + 1) * BQ] = oo
                ok = jnp.abs(oo) < jnp.inf
                ok8 = ok[0:8] & ok[8:16] & ok[16:24] & ok[24:32] & ok[32:40]
                okl = (l_e >= L_LO) & (l_e <= L_HI) & (l_o >= L_LO) & (l_o <= L_HI)
                bad = jnp.where(ok8 & okl, bad, 1.0)
        return bad

    bad = lax.fori_loop(0, H // 2, fast, jnp.zeros((8, BQ), f32))

    @pl.when(jnp.max(bad) > 0.0)
    def _():
        l32 = lax.broadcasted_iota(jnp.int32, (S, 32), 1)

        def pair(p, c):
            roll_keys(p, False)
            roll_keys(p, True)
            r0 = pl.multiple_of(p * (2 * DH), 8)

            def qblk(b, c2):
                c0 = pl.multiple_of(b * BQS, BQS)
                os_ = []
                for e in range(2):
                    lo = 4 * e
                    kh = kr_v[e, :, 0:32].astype(f32)
                    kh = jnp.where((l32 >= lo) & (l32 < lo + DH), kh, 0.0).astype(bf16)
                    s = _mm(kh, qt_v[2 * p + e, :, pl.ds(c0, BQS)])
                    m = jnp.max(s, axis=0, keepdims=True)
                    pt = jnp.exp2(s - m).astype(bf16)
                    os_.append(_mm(vt_v[2 * p + e], pt))
                oo, _, _ = merge(os_[0], os_[1])
                ot_v[pl.ds(r0, 2 * DH), pl.ds(c0, BQS)] = oo
                return c2

            return lax.fori_loop(0, S // BQS, qblk, c)

        lax.fori_loop(0, H // 2, pair, 0)

    for c in cp_rest:
        c.wait()

    def out_copy(i):
        r0 = pl.multiple_of(i * RB3, RB3)
        return pltpu.make_async_copy(
            out_v.at[pl.ds(r0, RB3)], out_hbm.at[pl.ds(r0, RB3)], out_sems.at[i])

    def p3(i, carry):
        r0 = pl.multiple_of(i * RB3, RB3)
        o = ot_v[:, pl.ds(r0, RB3)].T.astype(bf16)
        h = x_v[pl.ds(r0, RB3), :].astype(f32) + _mm(o, wo_v[...])
        hn = _layernorm(h).astype(bf16)
        g = _mm(hn, wg_v[...])
        u = _mm(hn, wu_v[...])
        a = (g * jax.nn.sigmoid(g) * u).astype(bf16)
        out_v[pl.ds(r0, RB3), :] = (h + _mm(a, wd_v[...])).astype(out_v.dtype)
        out_copy(i).start()
        return carry

    lax.fori_loop(0, S // RB3, p3, 0)
    for i in range(S // RB3):
        out_copy(i).wait()


@jax.jit
def pallas_sequential_preLN__mha_block__swiglu_ffn__prompt_kernel(
    A_x: jax.Array,
    A_wqkv: jax.Array,
    A_wo: jax.Array,
    B_x: jax.Array,
    B_w_gate: jax.Array,
    B_w_up: jax.Array,
    B_w_down: jax.Array,
):
    del B_x
    B, S, D = A_x.shape
    F = B_w_gate.shape[1]
    any_spec = pl.BlockSpec(memory_space=pl.ANY)
    out = pl.pallas_call(
        _kernel,
        out_shape=jax.ShapeDtypeStruct((S, D), A_x.dtype),
        in_specs=[any_spec] * 6,
        out_specs=any_spec,
        scratch_shapes=[
            pltpu.VMEM((S, D), A_x.dtype),
            pltpu.VMEM((D, 3 * D), A_wqkv.dtype),
            pltpu.VMEM((D, D), A_wo.dtype),
            pltpu.VMEM((D, F), B_w_gate.dtype),
            pltpu.VMEM((D, F), B_w_up.dtype),
            pltpu.VMEM((F, D), B_w_down.dtype),
            pltpu.VMEM((2 * D, D), bf16),
            pltpu.VMEM((D // 128, S, 128), bf16),
            pltpu.VMEM((H, 32, S), bf16),
            pltpu.VMEM((H, 24, S), f32),
            pltpu.VMEM((2, S, 128), bf16),
            pltpu.VMEM((D, S), f32),
            pltpu.VMEM((S, D), A_x.dtype),
            pltpu.SemaphoreType.DMA((6,)),
            pltpu.SemaphoreType.DMA((S // RB3,)),
        ],
        compiler_params=pltpu.CompilerParams(vmem_limit_bytes=100 * 1024 * 1024),
    )(A_x.reshape(S, D), A_wqkv, A_wo, B_w_gate, B_w_up, B_w_down)
    return out.reshape(B, S, D)
```

```python
import jax
import jax.numpy as jnp
from jax import lax
import jax.experimental.pallas as pl
import jax.experimental.pallas.tpu as pltpu

H = 32
DH = 20
EPS = 1e-5
LOG2E = 1.4426950408889634
L_LO = 2.0 ** -30
L_HI = 2.0 ** 60

RB1 = 512
RB3 = 128
BQ = 512
KC = 256
PU = 2
FC = 896
LA = 1
BQS = 256

f32 = jnp.float32
bf16 = jnp.bfloat16


def _mm(a, b):
    return lax.dot_general(a, b, (((1,), (0,)), ((), ())), preferred_element_type=f32)


def _mm_nt(a, b):
    return lax.dot_general(a, b, (((1,), (1,)), ((), ())), preferred_element_type=f32)


def _layernorm(x):
    m = jnp.mean(x, axis=-1, keepdims=True)
    d = x - m
    v = jnp.mean(d * d, axis=-1, keepdims=True)
    return d * lax.rsqrt(v + EPS)


def _kernel(x_hbm, wqkv_hbm, wo_hbm, wg_hbm, wu_hbm, wd_hbm, out_hbm,
            x_v, wqkv_v, wo_v, wgu_v, wd_v,
            wqvt_v, kr_v, qt_v, vt_v, ot_v, out_v,
            x_sems, w_sems, r_sems, out_sems):
    S, D = x_v.shape
    F = wd_v.shape[0]
    FA = F // 128 * 128
    FT = F - FA
    assert FT == 64

    cp_x = [pltpu.make_async_copy(x_hbm.at[i * RB1:(i + 1) * RB1],
                                  x_v.at[i * RB1:(i + 1) * RB1], x_sems.at[i])
            for i in range(S // RB1)]
    cp_w = [pltpu.make_async_copy(wqkv_hbm.at[:, i * D:(i + 1) * D],
                                  wqkv_v.at[i], w_sems.at[i]) for i in range(3)]
    cp_rest = [
        pltpu.make_async_copy(wo_hbm, wo_v, r_sems.at[0]),
        pltpu.make_async_copy(wg_hbm.at[0:FA], wgu_v.at[0:FA], r_sems.at[1]),
        pltpu.make_async_copy(wu_hbm.at[0:FA], wgu_v.at[FA:2 * FA], r_sems.at[2]),
        pltpu.make_async_copy(wg_hbm.at[FA:F], wgu_v.at[2 * FA:2 * FA + FT], r_sems.at[3]),
        pltpu.make_async_copy(wu_hbm.at[FA:F], wgu_v.at[2 * FA + FT:2 * F], r_sems.at[4]),
        pltpu.make_async_copy(wd_hbm, wd_v, r_sems.at[5]),
    ]
    cp_x[0].start()
    cp_w[1].start()

    qscale = (DH ** -0.5) * LOG2E
    row8 = lax.broadcasted_iota(jnp.int32, (8, RB1), 0)

    lane = lax.broadcasted_iota(jnp.int32, (RB1 // 2, 128), 1)

    def p1_k(xn):
        return pltpu.bitcast(_mm(xn, wqkv_v[1]).astype(bf16), jnp.uint32)

    def p1_kwin(i, k):
        for h in range(H):
            t, off = divmod(DH * h - 4 * (h % 2), 128)
            kw = k[:, t * 128:(t + 1) * 128]
            if off + 24 > 128:
                kw = jnp.where(lane >= off, kw, k[:, (t + 1) * 128:(t + 2) * 128])
            if off:
                kw = pltpu.roll(kw, 128 - off, 1)
            kr_v[h, i * RB1:(i + 1) * RB1, :] = pltpu.bitcast(kw, bf16)

    def p1_q(i, xn):
        cs = slice(i * RB1, (i + 1) * RB1)
        qt = _mm_nt(wqvt_v[0:D, :], xn) * qscale
        zeros8 = jnp.zeros((8, RB1), f32)
        for p in range(H // 2):
            a = 2 * DH * p
            q_mid = qt[a + 16:a + 24]
            q_even = jnp.concatenate(
                [qt[a:a + 16], jnp.where(row8 < 4, q_mid, 0.0), zeros8], axis=0)
            q_odd = jnp.concatenate(
                [jnp.where(row8 >= 4, q_mid, 0.0), qt[a + 24:a + 40], zeros8], axis=0)
            qt_v[2 * p, :, cs] = q_even.astype(bf16)
            qt_v[2 * p + 1, :, cs] = q_odd.astype(bf16)

    def p1_v(i, xn):
        cs = slice(i * RB1, (i + 1) * RB1)
        vt = _mm_nt(wqvt_v[D:2 * D, :], xn)
        for p in range(H // 2):
            a = 2 * DH * p
            v_mid = vt[a + 16:a + 24]
            vt_v[2 * p, :, cs] = jnp.concatenate(
                [vt[a:a + 16], jnp.where(row8 < 4, v_mid, 1.0)], axis=0)
            vt_v[2 * p + 1, :, cs] = jnp.concatenate(
                [jnp.where(row8 >= 4, v_mid, 1.0), vt[a + 24:a + 40]], axis=0)

    def ln1(i):
        return _layernorm(x_v[i * RB1:(i + 1) * RB1, :].astype(f32)).astype(bf16)

    cp_x[0].wait()
    cp_x[1].start()
    cp_w[0].start()
    cp_w[2].start()
    xn0 = ln1(0)
    cp_w[1].wait()
    k0 = p1_k(xn0)
    cp_x[1].wait()
    cp_w[0].wait()
    for c in cp_x[2:]:
        c.start()
    xn1 = ln1(1)
    k1 = p1_k(xn1)
    wqvt_v[0:D, :] = wqkv_v[0].T
    cp_w[2].wait()
    for c in cp_x[2:]:
        c.wait()
    for c in cp_rest:
        c.start()
    p1_q(0, xn0)
    wqvt_v[D:2 * D, :] = wqkv_v[2].T
    p1_kwin(0, k0)
    p1_q(1, xn1)
    xns = [xn0, xn1] + [ln1(i) for i in range(2, S // RB1)]
    p1_v(0, xn0)
    p1_kwin(1, k1)
    p1_v(1, xn1)
    for i in range(2, S // RB1):
        p1_kwin(i, p1_k(xns[i]))
        p1_q(i, xns[i])
        p1_v(i, xns[i])

    def merge(o_e, o_o):
        l_e = o_e[20:21]
        l_o = o_o[0:1]
        n_e = o_e * (1.0 / l_e)
        n_o = o_o * (1.0 / l_o)
        r8 = lax.broadcasted_iota(jnp.int32, (8, o_e.shape[1]), 0)
        mid = jnp.where(r8 < 4, n_e[16:24], n_o[0:8])
        o = jnp.concatenate([n_e[0:16], mid, n_o[8:24]], axis=0)
        return o, l_e, l_o

    def fast(g, bad):
        nk = S // KC
        items = [(pp, qb, e, j) for pp in range(PU) for qb in range(S // BQ)
                 for e in range(2) for j in range(nk)]

        def scores(it):
            pp, qb, e, j = it
            h = 2 * (g * PU + pp) + e
            return _mm(kr_v[h, j * KC:(j + 1) * KC, 0:32], qt_v[h, :, qb * BQ:(qb + 1) * BQ])

        pending = [scores(it) for it in items[:LA]]
        accs = {}
        for n, (pp, qb, e, j) in enumerate(items):
            if n + LA < len(items):
                pending.append(scores(items[n + LA]))
            pt = jnp.exp2(pending.pop(0)).astype(bf16)
            o = _mm(vt_v[2 * (g * PU + pp) + e, :, j * KC:(j + 1) * KC], pt)
            accs[e] = o if j == 0 else accs[e] + o
            if e == 1 and j == nk - 1:
                oo, l_e, l_o = merge(accs[0], accs[1])
                r0 = pl.multiple_of((g * PU + pp) * (2 * DH), 8)
                ot_v[pl.ds(r0, 2 * DH), qb * BQ:(qb + 1) * BQ] = oo
                ok = jnp.abs(oo) < jnp.inf
                ok8 = ok[0:8] & ok[8:16] & ok[16:24] & ok[24:32] & ok[32:40]
                okl = (l_e >= L_LO) & (l_e <= L_HI) & (l_o >= L_LO) & (l_o <= L_HI)
                bad = jnp.where(ok8 & okl, bad, 1.0)
        return bad

    bad = lax.fori_loop(0, H // 2 // PU, fast, jnp.zeros((8, BQ), f32))

    @pl.when(jnp.max(bad) > 0.0)
    def _():
        l32 = lax.broadcasted_iota(jnp.int32, (S, 32), 1)

        def step(t, c):
            p = t // (S // BQS)
            r0 = pl.multiple_of(p * (2 * DH), 8)
            c0 = pl.multiple_of((t % (S // BQS)) * BQS, BQS)
            os_ = []
            for e in range(2):
                lo = 4 * e
                kh = kr_v[2 * p + e, :, 0:32].astype(f32)
                kh = jnp.where((l32 >= lo) & (l32 < lo + DH), kh, 0.0).astype(bf16)
                s = _mm(kh, qt_v[2 * p + e, :, pl.ds(c0, BQS)])
                m = jnp.max(s, axis=0, keepdims=True)
                pt = jnp.exp2(s - m).astype(bf16)
                os_.append(_mm(vt_v[2 * p + e], pt))
            oo, _, _ = merge(os_[0], os_[1])
            ot_v[pl.ds(r0, 2 * DH), pl.ds(c0, BQS)] = oo
            return c

        lax.fori_loop(0, (H // 2) * (S // BQS), step, 0)

    for c in cp_rest:
        c.wait()

    def out_copy(i):
        rs = slice(i * RB3, (i + 1) * RB3)
        return pltpu.make_async_copy(out_v.at[rs], out_hbm.at[rs], out_sems.at[i])

    def attn_out(i):
        rs = slice(i * RB3, (i + 1) * RB3)
        o = ot_v[:, rs].astype(bf16).T
        h = x_v[rs, :].astype(f32) + _mm(o, wo_v[...])
        return h, _layernorm(h).astype(bf16)

    def act(hn, c0, c1):
        if c0 == FA:
            t = _mm_nt(hn, wgu_v[2 * FA:2 * F, :])
            return (t * jax.nn.sigmoid(t) * pltpu.roll(t, FT, 1))[:, 0:FT].astype(bf16)
        g = _mm_nt(hn, wgu_v[c0:c1, :])
        u = _mm_nt(hn, wgu_v[FA + c0:FA + c1, :])
        return (g * jax.nn.sigmoid(g) * u).astype(bf16)

    chunks = [(FA, F)] + [(c, min(c + FC, FA)) for c in range(0, FA, FC)]
    nb = S // RB3
    h, hn = attn_out(0)
    for i in range(nb):
        acc = h
        a = act(hn, *chunks[0])
        for n, (c0, c1) in enumerate(chunks):
            if n + 1 < len(chunks):
                a_next = act(hn, *chunks[n + 1])
            if n == len(chunks) - 2 and i + 1 < nb:
                h, hn = attn_out(i + 1)
            acc = acc + _mm(a, wd_v[c0:c1, :])
            a = a_next
        out_v[i * RB3:(i + 1) * RB3, :] = acc.astype(out_v.dtype)
        out_copy(i).start()
    for i in range(nb):
        out_copy(i).wait()


@jax.jit
def pallas_sequential_preLN__mha_block__swiglu_ffn__prompt_kernel(
    A_x: jax.Array,
    A_wqkv: jax.Array,
    A_wo: jax.Array,
    B_x: jax.Array,
    B_w_gate: jax.Array,
    B_w_up: jax.Array,
    B_w_down: jax.Array,
):
    del B_x
    B, S, D = A_x.shape
    F = B_w_gate.shape[1]
    any_spec = pl.BlockSpec(memory_space=pltpu.HBM)
    out = pl.pallas_call(
        _kernel,
        out_shape=jax.ShapeDtypeStruct((S, D), A_x.dtype),
        in_specs=[any_spec] * 6,
        out_specs=any_spec,
        scratch_shapes=[
            pltpu.VMEM((S, D), A_x.dtype),
            pltpu.VMEM((3, D, D), A_wqkv.dtype),
            pltpu.VMEM((D, D), A_wo.dtype),
            pltpu.VMEM((2 * F, D), B_w_gate.dtype),
            pltpu.VMEM((F, D), B_w_down.dtype),
            pltpu.VMEM((2 * D, D), bf16),
            pltpu.VMEM((H, S, 128), bf16),
            pltpu.VMEM((H, 32, S), bf16),
            pltpu.VMEM((H, 24, S), f32),
            pltpu.VMEM((D, S), f32),
            pltpu.VMEM((S, D), A_x.dtype),
            pltpu.SemaphoreType.DMA((S // RB1,)),
            pltpu.SemaphoreType.DMA((3,)),
            pltpu.SemaphoreType.DMA((6,)),
            pltpu.SemaphoreType.DMA((S // RB3,)),
        ],
        compiler_params=pltpu.CompilerParams(vmem_limit_bytes=100 * 1024 * 1024),
    )(A_x.reshape(S, D), A_wqkv, A_wo, B_w_gate.T, B_w_up.T, B_w_down)
    return out.reshape(B, S, D)
```
